```python
import os as _os
_os.environ.setdefault("JAX_PLATFORMS", "cpu")
import jax
import jax.numpy as jnp

def _softmax(x, axis=-1):
    return jax.nn.softmax(x, axis=axis)
def _gelu(x):
    return jax.nn.gelu(x, approximate=True)
def _silu(x):
    return jax.nn.silu(x)
def _sigmoid(x):
    return jax.nn.sigmoid(x)
def _layernorm(x, axis=-1, eps=1e-5):
    m = jnp.mean(x, axis=axis, keepdims=True)
    v = jnp.var(x, axis=axis, keepdims=True)
    return (x - m) / jnp.sqrt(v + eps)
def _scatter_add(tgt, idx, src, axis=0):
    return tgt.at[idx].add(src)
def _segment_sum(src, seg, n):
    return jax.ops.segment_sum(src, seg, n)
class _Rng:
    def __init__(self, key):
        self._k = key
    def _next(self):
        self._k, sub = jax.random.split(self._k)
        return sub
    def normal(self, shape):
        return jax.random.normal(self._next(), shape, dtype=jnp.bfloat16)
    def randint(self, lo, hi, shape):
        return jax.random.randint(self._next(), shape, lo, hi, dtype=jnp.int32)
    def uniform(self, shape, lo=0.0, hi=1.0):
        return jax.random.uniform(self._next(), shape, jnp.bfloat16, lo, hi)
    def permutation(self, n):
        return jax.random.permutation(self._next(), n)


kernel_name = 'sequential_preLN__sliding_block__dense_activation_gelu__prompt'

def setup_inputs():
    _rng = _Rng(jax.random.key(int.from_bytes(__import__("os").urandom(4), "little")))
    _w = (lambda a: (lambda t: t.astype(jnp.bfloat16) if jnp.issubdtype(t.dtype, jnp.floating) else t)(jnp.asarray(a)))
    def _A_setup():
        B, S, D = 1, 2048, 640
        return {
            "x": _w((lambda *s: _rng.normal(s) * 0.05)(B, S, D)),
            "wqkv": _w((lambda *s: _rng.normal(s) * 0.05)(D, 3 * D)),
            "wo": _w((lambda *s: _rng.normal(s) * 0.05)(D, D)),
        }
    _A_in = _A_setup()

    def _B_setup():
        B, S, D, F = 1, 2048, 640, 1536
        return {
            "x": _w((lambda *s: _rng.normal(s) * 0.05)(B, S, D)),
            "w1": _w((lambda *s: _rng.normal(s) * 0.8)(D, F) * (D ** -0.5)),
            "b1": _w((lambda *s: _rng.normal(s) * 0.8)(F) * 0.01),
            "w2": _w((lambda *s: _rng.normal(s) * 0.8)(F, D) * (F ** -0.5)),
            "b2": _w((lambda *s: _rng.normal(s) * 0.05)(D) * 0.01),
        }
    _B_in = _B_setup()

    return {
        "A_x": _A_in["x"],
        "A_wqkv": _A_in["wqkv"],
        "A_wo": _A_in["wo"],
        "B_x": _B_in["x"],
        "B_w1": _B_in["w1"],
        "B_b1": _B_in["b1"],
        "B_w2": _B_in["w2"],
        "B_b2": _B_in["b2"],
    }

def reference(A_x, A_wqkv, A_wo, B_x, B_w1, B_b1, B_w2, B_b2):
    def _A_ref(x, wqkv, wo):
        B, S, D = x.shape
        H = 32; Dh = D // H; W = 256
        qkv = (lambda x, *d: x.transpose(*d))((x @ wqkv).reshape(B, S, 3, H, Dh), 2, 0, 3, 1, 4)
        q, k, v = qkv[0], qkv[1], qkv[2]
        scores = jnp.einsum("bhqd,bhkd->bhqk", q, k) * (Dh ** -0.5)
        idx = jnp.arange(S)
        mask = (idx[:, None] - idx[None, :] >= 0) & (idx[:, None] - idx[None, :] < W)
        scores = jnp.where(mask[None, None], scores, -1e9)
        p = _softmax(scores, axis=-1)
        o = jnp.einsum("bhqk,bhkd->bhqd", p, v)
        return (lambda x, *d: x.transpose(*d))(o, 0, 2, 1, 3).reshape(B, S, D) @ wo

    def _B_ref(x, w1, b1, w2, b2):
        h = jnp.einsum("bsd,df->bsf", x, w1) + b1
        h = _gelu(h)
        return jnp.einsum("bsf,fd->bsd", h, w2) + b2

    x = A_x
    h = x + _A_ref(_layernorm(x, axis=-1), A_wqkv, A_wo)
    h2 = h + _B_ref(_layernorm(h, axis=-1), B_w1, B_b1, B_w2, B_b2)
    return h2
```

```python
import functools
import math

import jax
import jax.numpy as jnp
import jax.experimental.pallas as pl
import jax.experimental.pallas.tpu as pltpu

H = 32
W = 256
T = 128
U = 64
TQ = 256
C = 256
R = 16
G = 4
PACE = (None, 0, 48, 112)
EPS = 1e-5
NEG = -1e30

f32, bf16 = jnp.float32, jnp.bfloat16


def _ln(x):
    m = jnp.mean(x, axis=-1, keepdims=True)
    c = x - m
    v = jnp.mean(c * c, axis=-1, keepdims=True)
    return c * jax.lax.rsqrt(v + EPS)


def _gelu(x):
    c1 = math.sqrt(2.0 / math.pi)
    c2 = c1 * 0.044715
    t = jnp.tanh(x * (c1 + c2 * (x * x)))
    hx = 0.5 * x
    return hx + hx * t


def _dot(a, b):
    return jax.lax.dot_general(a, b, (((1,), (0,)), ((), ())), preferred_element_type=f32)


def _lhs_sums(a11, a12, a21, a22):
    return (a11 + a22, a21 + a22, a11, a22, a11 + a12, a21 - a11, a12 - a22)


def _rhs_sums(b11, b12, b21, b22):
    return (b11 + b22, b12 - b22, b21 - b11, b11 + b12, b21 + b22)


def _put(ref, i, j0, val):
    for j in range(val.shape[1] // T):
        ref[i, j0 + j] = val[:, j * T:(j + 1) * T].astype(bf16)


def _get(ref, i, j0=0, n=None):
    n = ref.shape[1] if n is None else n
    return jnp.concatenate([ref[i, j0 + j] for j in range(n)], axis=1)


def _quadrants(a, w, b11, b22, e, post):
    n = b11.shape[1]
    el, er = e[:, :n], e[:, n:]
    m3 = _dot(a(2), w(1))
    m5 = _dot(a(4), b22)
    c12 = post(er[:T] + m3 + m5)
    m2 = _dot(a(1), b11)
    m4 = _dot(a(3), w(2))
    c21 = post(el[T:] + m2 + m4)
    m1 = _dot(a(0), w(0))
    m6 = _dot(a(5), w(3))
    c22 = post(er[T:] + m3 - m2 + m1 + m6)
    m7 = _dot(a(6), w(4))
    c11 = post(el[:T] - m5 + m4 + m1 + m7)
    return c11, c12, c21, c22


def _kernel(x_hbm, wqkv_hbm, wo_hbm, w1_hbm, b1_hbm, w2_hbm, b2_hbm, o_hbm,
            x_scr, o_scr, wqkv_scr, wo_scr, w1_scr, w2_scr,
            xn_scr, kc_scr, k_scr, vt_scr, qt_scr, ot_scr, msk_scr, zero_scr, qm_scr, s_scr, p_scr,
            h_scr, hn_scr, a_scr, xs_scr, wqs_scr, w1s_scr, w2s_scr, g_scr, b1_ref, b2_ref,
            xsem, osem, wsem):
    S, D = x_hbm.shape
    Dh = D // H
    ND = D // T
    NQ = TQ // T
    NG = H // G
    NB = S // TQ
    assert (D, Dh, W, TQ) == (5 * T, 20, 2 * T, 2 * T) and S % TQ == 0 and NB >= 3

    def rows(b, lo=0, n=TQ):
        if isinstance(b, int):
            return pl.ds(b * TQ + lo, n)
        return pl.ds(pl.multiple_of(b * TQ + lo, n), n)

    def x_copy(b):
        return pltpu.make_async_copy(x_hbm.at[rows(b)], x_scr.at[rows(b)], xsem.at[b])

    def o_copy(b):
        return pltpu.make_async_copy(o_scr.at[rows(b)], o_hbm.at[rows(b)], osem.at[b])

    def last_copy(j):
        cols = (slice(0, 2 * C), slice(2 * C, D))[j]
        return pltpu.make_async_copy(o_scr.at[rows(NB - 1), cols], o_hbm.at[rows(NB - 1), cols],
                                     osem.at[NB - 1 + j])

    def wqkv_copy(j):
        sl = pl.ds(j * D, D)
        return pltpu.make_async_copy(wqkv_hbm.at[:, sl], wqkv_scr.at[j], wsem.at[j])

    b1_copy = pltpu.make_async_copy(b1_hbm, b1_ref, wsem.at[6])
    b2_copy = pltpu.make_async_copy(b2_hbm, b2_ref, wsem.at[7])
    wo_copy = pltpu.make_async_copy(wo_hbm, wo_scr, wsem.at[3])
    w1_copy = pltpu.make_async_copy(w1_hbm, w1_scr, wsem.at[4])
    w2_copy = pltpu.make_async_copy(w2_hbm, w2_scr, wsem.at[5])

    def ln1(b, split=True):
        y = _ln(x_scr[rows(b), :].astype(f32))
        xn_scr[...] = y.astype(bf16)
        if split:
            for i, a in enumerate(_lhs_sums(y[:T, :C], y[:T, C:2 * C], y[T:, :C], y[T:, C:2 * C])):
                if i not in (2, 3):
                    _put(xs_scr, i, 0, a)

    LEFT = [(1, j) for j in range(ND)] + [(2, 0), (2, 1)]
    RIGHT = [(0, j) for j in range(ND)] + [(2, 2), (2, 3)]

    def wtiles(tiles, r0, n):
        return jnp.concatenate([wqkv_scr[m, r0:r0 + n, j * T:(j + 1) * T] for m, j in tiles], axis=1)

    def sum_job(src, dst, j, z):
        def job(dep):
            zero = zero_scr[...] & pltpu.bitcast(dep, jnp.int32)
            q = src()
            for i in (0, 3):
                q[i] = pltpu.bitcast(pltpu.bitcast(q[i], jnp.int32) | zero, bf16)
            for i, w in enumerate(_rhs_sums(*[v.astype(f32) for v in q])):
                dst[i, j, z:z + R] = w.astype(bf16)
        return job

    def pace(jobs, vals):
        deps = [v[r:r + 8, c:c + T] for v in vals
                for c in range(0, v.shape[1], T) for r in range(0, v.shape[0], 8)]
        for i, job in enumerate(jobs):
            job(deps[i * len(deps) // len(jobs)])

    def wqkv_sums(*js):
        src = lambda j, z: lambda: [wtiles(t[j:j + 1], r + z, R) for r in (0, C) for t in (LEFT, RIGHT)]
        return [sum_job(src(j, z), wqs_scr, j, z) for j in js for z in range(0, C, R)]

    def w1_sums(*js):
        n = w1_scr.shape[1] // 2
        src = lambda j, z: lambda: [w1_scr[r + z:r + z + R, c + j * T:c + (j + 1) * T]
                                    for r in (0, C) for c in (0, n)]
        return [sum_job(src(j, z), w1s_scr, j, z) for j in js for z in range(0, C, R)]

    def w2_sums(*zs):
        n = w2_scr.shape[0] // 2
        src = lambda j, z: lambda: [w2_scr[r + z:r + z + R, c + j * T:c + (j + 1) * T]
                                    for r in (0, n) for c in (0, C)]
        return [sum_job(src(j, z), w2s_scr, j, z)
                for y in zs for j in range(C // T) for z in range(y * T, (y + 1) * T, R)]

    def qkv_pieces(b):
        scale = (Dh ** -0.5) * math.log2(math.e)
        a = lambda i: xn_scr[:T, :C] if i == 2 else xn_scr[T:, C:2 * C] if i == 3 else _get(xs_scr, i)
        k = {}

        def emit(m, j, i, val):
            if m == 0:
                qt_scr[j * T:(j + 1) * T, i * T:(i + 1) * T] = (val * scale).T.astype(bf16)
            elif m == 1:
                k[j, i] = val
            else:
                vt_scr[b * NQ + i, j * T:(j + 1) * T] = val.T

        def chunk(c, jobs=()):
            l, r = LEFT[c:c + 2], RIGHT[c:c + 2]
            e = _dot(xn_scr[:, 2 * C:], wtiles(l + r, 2 * C, D - 2 * C))
            cs = _quadrants(a, lambda i: _get(wqs_scr, i, c, len(l)), wtiles(l, 0, C), wtiles(r, C, C), e, lambda v: v)
            pace(jobs, [cs[1], cs[2], cs[3], cs[0]])
            for z, val in enumerate(cs):
                for y, (m, j) in enumerate(r if z % 2 else l):
                    emit(m, j, z // 2, val[:, y * T:(y + 1) * T])
            if (1, ND - 1) in l:
                put_k(b, jnp.concatenate(
                    [jnp.concatenate([k[j, i] for j in range(ND)], axis=1) for i in range(NQ)], axis=0))

        def rest(jobs=()):
            v = _dot(xn_scr[...], wtiles([(2, ND - 1)], 0, D))
            pace(jobs, [v])
            for i in range(NQ):
                emit(2, ND - 1, i, v[i * T:(i + 1) * T])

        return [functools.partial(chunk, c) for c in range(0, len(LEFT), 2)] + [rest]

    def proj(j):
        return _dot(xn_scr[...], wqkv_scr[j])

    def put_q(q):
        qt_scr[...] = (q * ((Dh ** -0.5) * math.log2(math.e))).T.astype(bf16)

    def put_k(b, k):
        first = isinstance(b, int) and b == 0
        kd = jnp.concatenate([jnp.zeros((U, D), f32) if first else kc_scr[...], k[:TQ - U]], axis=0)
        kc_scr[...] = k[TQ - U:]
        lane = jax.lax.broadcasted_iota(jnp.int32, (TQ, T), 1)
        lo = [kd[:, j * T:(j + 1) * T] for j in range(ND)]
        hi = [pltpu.roll(k[:, j * T:(j + 1) * T], U, 1) for j in range(ND)]
        for p in range(H // 2):
            a0 = p * 2 * Dh
            j0, j1 = a0 // T, (a0 + 2 * Dh - 1) // T
            l0 = a0 % T
            if j0 == j1:
                kp = jnp.where((lane >= l0) & (lane < l0 + 2 * Dh), lo[j0], hi[j0])
            else:
                kp = jnp.where(lane < U, jnp.where(lane < l0 + 2 * Dh - T, lo[j1], hi[j0]),
                               jnp.where(lane < l0, hi[j1], lo[j0]))
            k_scr[p, rows(b), :] = kp.astype(bf16)

    def put_v(b, v):
        vt = v.T
        for i in range(NQ):
            vt_scr[b * NQ + i] = vt[:, i * T:(i + 1) * T]

    def attention(b, *fills):
        r = jax.lax.broadcasted_iota(jnp.int32, (U, T), 0)
        c = jax.lax.broadcasted_iota(jnp.int32, (U, T), 1)
        tri = r <= (c & (U - 1))
        c32 = jax.lax.broadcasted_iota(jnp.int32, (32, T), 1)
        r8 = jax.lax.broadcasted_iota(jnp.int32, (8, T), 0)
        units = [(i, g) for i in range(NQ) for g in range(NG)]

        def ntiles(i):
            return min(3, b * NQ + i + 1) if isinstance(b, int) else 3

        def window(h):
            d0 = h * Dh
            w0 = (d0 // 16) * 16
            return w0, d0 - w0

        def qk(u):
            i, g = units[u]
            nt = ntiles(i)
            nb = min(2 * nt, 5)
            k0 = b * TQ + (i + 1) * T - nb * U
            if not isinstance(b, int):
                k0 = pl.multiple_of(k0, U)
            ms, ss = [], []
            for p in range(g * G // 2, (g + 1) * G // 2):
                ws = []
                for h in (2 * p, 2 * p + 1):
                    w0, off = window(h)
                    qw = pltpu.bitcast(qt_scr[w0:w0 + 32, i * T:(i + 1) * T], jnp.int32)
                    q_lo = pltpu.bitcast(qw & qm_scr[off // 2], bf16)
                    q_hi = pltpu.bitcast(qw & qm_scr[off // 2 + 1], bf16)
                    parts = [jnp.zeros((16, T), bf16)] * (T // 16)
                    p0 = (w0 % T) // 16
                    for z in range(2):
                        parts[(p0 + z) % 8] = q_lo[16 * z:16 * z + 16]
                        parts[(p0 + z + 4) % 8] = q_hi[16 * z:16 * z + 16]
                    ws.append(jnp.concatenate(parts, axis=0))
                s = _dot(k_scr[p, pl.ds(k0, nb * U), :], jnp.concatenate(ws, axis=1))
                for jj in range(2):
                    j = len(ms)
                    sj = s[:, jj * T:(jj + 1) * T]
                    ss.append(sj)
                    s_a = jnp.where(tri, sj[(nb - 1) * U:], sj[0:U] if nb == 5 else NEG)
                    s_scr[u % 2, j, 3] = s_a
                    for z in range(1, min(nb, 4)):
                        s_b = sj[(nb - 1 - z) * U:(nb - z) * U]
                        if nb < 5 and z == nb - 1:
                            s_b = jnp.where(c >= U, s_b, NEG)
                        s_scr[u % 2, j, 3 - z] = s_b
                        s_a = jnp.maximum(s_a, s_b)
                    ms.append(jnp.max(s_a, axis=0, keepdims=True))
            return ms, ss

        def sm(u, ms):
            nb = min(2 * ntiles(units[u][0]), 5)
            for j in range(G):
                for z in range(4 - min(nb, 4), 4):
                    p_scr[u % 2, j, z] = jnp.exp2(s_scr[u % 2, j, z] - ms[j]).astype(bf16)

        def pv(u):
            i, g = units[u]
            nt = ntiles(i)
            nb = min(2 * nt, 5)
            r8w = jax.lax.broadcasted_iota(jnp.int32, (8, nt * T), 0)
            left = c32 < U
            os_ = []
            for j in range(G):
                ps = [pltpu.bitcast(p_scr[u % 2, j, z], jnp.int32) for z in range(4 - min(nb, 4), 4)]
                if nb == 5:
                    cur = ps[3] & msk_scr[...]
                    ps = [ps[3] ^ cur, ps[0], ps[1], ps[2], cur]
                    pk = [jnp.where(left, ps[0], 0)]
                else:
                    pk = []
                pk += [jnp.where(left, ps[z + 1], ps[z]) for z in range(len(ps) - 1)]
                pk += [jnp.where(left, 0, ps[-1])]
                p = pltpu.bitcast(jnp.concatenate(pk, axis=0), bf16)
                t0 = b * NQ + i + 1 - nt
                h = g * G + j
                v0 = (h * Dh // 8) * 8
                vw = jnp.concatenate([vt_scr[t0 + t, v0:v0 + 24, :] for t in range(nt)], axis=1)
                if h % 2 == 0:
                    vw = jnp.concatenate([vw[0:16], jnp.where(r8w < 4, vw[16:24], 1.0)], axis=0)
                else:
                    vw = jnp.concatenate([jnp.where(r8w < 4, 1.0, vw[0:8]), vw[8:24]], axis=0)
                os_.append(_dot(vw, p))
            return os_

        def fin(u, os_):
            i, g = units[u]
            cols = slice(i * T, (i + 1) * T)
            for j in range(0, G, 2):
                a = os_[j] * (1.0 / os_[j][20:21, :])
                z = os_[j + 1] * (1.0 / os_[j + 1][0:1, :])
                g0 = (g * G + j) * Dh
                ot_scr[g0:g0 + 16, cols] = a[0:16]
                ot_scr[g0 + 16:g0 + 24, cols] = jnp.where(r8 < 4, a[16:24], z[0:8])
                ot_scr[g0 + 24:g0 + 40, cols] = z[8:24]

        n = len(units)

        def after(m, xs):
            z = zero_scr[0:1]
            for x in xs:
                z = z & pltpu.bitcast(x, jnp.int32)
            return pltpu.bitcast(pltpu.bitcast(m, jnp.int32) | z, f32)

        ms, ss, os_ = {}, {}, {}
        for t in range(n + 3):
            if t < n:
                ms[t], ss[t] = qk(t)
            if 0 <= t - 1 < n:
                m = ms.pop(t - 1)
                for j, row in enumerate(PACE):
                    if row == 0 and t >= 3:
                        m[j] = after(m[j], [x[16:17] for x in os_[t - 3]])
                    elif row and t < n and row <= ss[t][0].shape[0]:
                        m[j] = after(m[j], [x[row - 8:row - 7] for x in ss[t]])
            if 0 <= t - 3 < n:
                fin(t - 3, os_.pop(t - 3))
            if 0 <= t - 1 < n:
                sm(t - 1, m)
            if 0 <= t - 2 < n:
                os_[t - 2] = pv(t - 2)
            for fill in fills:
                if t in fill:
                    fill[t]()

    def heads():
        return ot_scr[...].T.astype(bf16)

    def proj_o(b, o, slot=0):
        h_scr[slot] = x_scr[rows(b), :].astype(f32) + _dot(o, wo_scr[...])

    def ln2(slot=0):
        y = _ln(h_scr[slot])
        for i, a in enumerate(_lhs_sums(y[:T, :C], y[:T, C:2 * C], y[T:, :C], y[T:, C:2 * C])):
            _put(a_scr, i, 0, a)
        hn_scr[...] = y[:, 2 * C:].astype(bf16)

    def ffn1():
        n = w1_scr.shape[1] // 2
        b1 = b1_ref[...].astype(f32)[None, :]
        for c in range(0, n, C):
            l, r = slice(c, c + C), slice(n + c, n + c + C)
            e = _dot(hn_scr[...], jnp.concatenate([w1_scr[2 * C:, l], w1_scr[2 * C:, r]], axis=1))
            e = e + jnp.concatenate([b1[:, l], b1[:, r]], axis=1)
            g11, g12, g21, g22 = _quadrants(
                lambda i: _get(a_scr, i), lambda i: _get(w1s_scr, i, c // T, 2),
                w1_scr[:C, l], w1_scr[C:2 * C, r], e, _gelu)
            for i, g in enumerate(_lhs_sums(g11, g12, g21, g22) + (g12, g21)):
                _put(g_scr, i, c // T, g)

    def ffn2_pieces(b, slot=0):
        n = w2_scr.shape[0] // 2
        m = {}

        def out(lo, c, val):
            nr, nc = val.shape
            cols = slice(c, c + nc)
            b2 = b2_ref[...].astype(f32)[None, :][:, cols]
            o_scr[rows(b, lo, nr), cols] = (h_scr[slot, lo:lo + nr, cols] + b2 + val).astype(o_scr.dtype)

        def product(i):
            a = _get(g_scr, i - 1)
            if i == 3:
                m[3] = _dot(a, _get(w2s_scr, 1))
            elif i == 5:
                m[5] = _dot(a, w2_scr[n:, C:2 * C])
                out(0, C, m[3] + m[5])
            elif i == 2:
                m[2] = _dot(a, w2_scr[:n, :C])
            elif i == 4:
                m[4] = _dot(a, _get(w2s_scr, 2))
                out(T, 0, m[2] + m[4])
                m[22], m[11] = m.pop(3) - m.pop(2), m.pop(4) - m.pop(5)
            elif i == 1:
                m[1] = _dot(a, _get(w2s_scr, 0))
            elif i == 6:
                out(T, C, m.pop(22) + m[1] + _dot(a, _get(w2s_scr, 3)))
            else:
                out(0, 0, m.pop(11) + m.pop(1) + _dot(a, _get(w2s_scr, 4)))

        def rest(kc):
            j = kc * C // T
            a = jnp.concatenate([
                jnp.concatenate([_get(g_scr, 2, j, 2), _get(g_scr, 7, j, 2)], axis=1),
                jnp.concatenate([_get(g_scr, 8, j, 2), _get(g_scr, 3, j, 2)], axis=1)], axis=0)
            w = jnp.concatenate([w2_scr[r + kc * C:r + (kc + 1) * C, 2 * C:] for r in (0, n)], axis=0)
            d = _dot(a, w)
            m[0] = d if kc == 0 else m[0] + d
            if kc == n // C - 1:
                out(0, 2 * C, m.pop(0))

        ps = [functools.partial(product, i) for i in (3, 5, 2, 4, 1, 6, 7)]
        return ps + [functools.partial(rest, kc) for kc in range(n // C)]

    x_copy(0).start()
    wqkv_copy(0).start()
    r = jax.lax.broadcasted_iota(jnp.int32, (U, T), 0)
    c = jax.lax.broadcasted_iota(jnp.int32, (U, T), 1)
    msk_scr[...] = pltpu.bitcast(jnp.where(r <= (c & (U - 1)), -1, 0).astype(jnp.int16), jnp.int32)
    r = jax.lax.broadcasted_iota(jnp.int32, (16, T), 0)
    c = jax.lax.broadcasted_iota(jnp.int32, (16, T), 1)
    zero_scr[...] = jnp.zeros((8, T), jnp.int32)
    for z in range(4):
        own = (r >= 2 * z) & (r < 2 * z + Dh // 2)
        qm_scr[2 * z] = jnp.where(own & (c < U), -1, 0)
        qm_scr[2 * z + 1] = jnp.where(own & (c >= U), -1, 0)
    x_copy(0).wait()
    wqkv_copy(1).start()
    ln1(0, False)
    wqkv_copy(0).wait()
    wqkv_copy(2).start()
    x_copy(1).start()
    q = proj(0)
    wqkv_copy(1).wait()
    w1_copy.start()
    k = []
    for j in range(ND):
        k.append(_dot(xn_scr[...], wtiles([(1, j)], 0, D)))
        if j == 0:
            put_q(q)
        if j < ND - 1:
            pace(wqkv_sums(j), k[-1:])
    wqkv_copy(2).wait()
    x_copy(1).wait()
    for c in (wo_copy, w2_copy, b1_copy, b2_copy):
        c.start()
    v = proj(2)
    put_k(0, jnp.concatenate(k, axis=1))
    ln1(1)
    pace(wqkv_sums(6), [v])
    put_v(0, v)
    qkv = qkv_pieces(1)
    attention(0, {2: qkv[4], 8: qkv[3], 16: lambda: qkv[0](wqkv_sums(4, 5))})
    for c in (w1_copy, wo_copy, w2_copy, b1_copy, b2_copy):
        c.wait()
    for b in range(2, NB):
        x_copy(b).start()
    qkv[1](w1_sums(0, 1, 2, 3))
    o = heads()
    x = x_scr[rows(0), :].astype(f32)
    for j in range(ND):
        cols = slice(j * T, (j + 1) * T)
        d = _dot(o, wo_scr[:, cols])
        h_scr[0, :, cols] = x[:, cols] + d
        pace(w2_sums(j) if j else w2_sums(0, 5), [d])
    ln2()
    qkv[2](w1_sums(4, 5))
    ffn1()

    def body(b, carry):
        x_copy(b + 1).wait()
        qkv = qkv_pieces(b + 1)
        fill = dict(zip((0, 2, 4, 6, 8, 10, 12, 14, 15, 16), ffn2_pieces(b - 1)))
        attention(b, fill, {8: lambda: ln1(b + 1)})
        proj_o(b, heads())
        qkv[4]()
        ln2()
        qkv[0]()
        qkv[1]()
        qkv[2]()
        qkv[3]()
        ffn1()
        o_copy(b - 1).start()
        return carry

    jax.lax.fori_loop(1, NB - 1, body, 0)

    b = NB - 1
    pieces = ffn2_pieces(b - 1)
    attention(b, dict(zip((1, 4, 7, 10, 13, 16, 17), pieces)))
    proj_o(b, heads(), 1)
    for piece in pieces[7:]:
        piece()
    ln2(1)
    o_copy(b - 1).start()
    ffn1()
    pieces = ffn2_pieces(b, 1)
    for piece in pieces[:8]:
        piece()
    last_copy(0).start()
    for piece in pieces[8:]:
        piece()
    last_copy(1).start()
    for b in range(NB - 1):
        o_copy(b).wait()
    last_copy(0).wait()
    last_copy(1).wait()


@jax.jit
def pallas_sequential_preLN__sliding_block__dense_activation_gelu__prompt_kernel(
    A_x: jax.Array,
    A_wqkv: jax.Array,
    A_wo: jax.Array,
    B_x: jax.Array,
    B_w1: jax.Array,
    B_b1: jax.Array,
    B_w2: jax.Array,
    B_b2: jax.Array,
):
    B, S, D = A_x.shape
    F = B_w1.shape[1]
    x = A_x.reshape(B * S, D)
    hbm = pl.BlockSpec(memory_space=pl.ANY)
    out = pl.pallas_call(
        _kernel,
        in_specs=[hbm] * 7,
        out_specs=hbm,
        out_shape=jax.ShapeDtypeStruct((S, D), A_x.dtype),
        scratch_shapes=[
            pltpu.VMEM((S, D), bf16),
            pltpu.VMEM((S, D), bf16),
            pltpu.VMEM((3, D, D), bf16),
            pltpu.VMEM((D, D), bf16),
            pltpu.VMEM((D, F), bf16),
            pltpu.VMEM((F, D), bf16),
            pltpu.VMEM((TQ, D), bf16),
            pltpu.VMEM((U, D), f32),
            pltpu.VMEM((H // 2, S, T), bf16),
            pltpu.VMEM((S // T, D, T), f32),
            pltpu.VMEM((D, TQ), bf16),
            pltpu.VMEM((D, TQ), f32),
            pltpu.VMEM((U // 2, T), jnp.int32),
            pltpu.VMEM((8, T), jnp.int32),
            pltpu.VMEM((8, 16, T), jnp.int32),
            pltpu.VMEM((2, G, 4, U, T), f32),
            pltpu.VMEM((2, G, 4, U, T), bf16),
            pltpu.VMEM((2, TQ, D), f32),
            pltpu.VMEM((TQ, D - 2 * C), bf16),
            pltpu.VMEM((7, C // T, T, T), bf16),
            pltpu.VMEM((7, C // T, T, T), bf16),
            pltpu.VMEM((5, 7, C, T), bf16),
            pltpu.VMEM((5, F // 2 // T, C, T), bf16),
            pltpu.VMEM((5, C // T, F // 2, T), bf16),
            pltpu.VMEM((9, F // 2 // T, T, T), bf16),
            pltpu.VMEM((F,), bf16),
            pltpu.VMEM((D,), bf16),
            pltpu.SemaphoreType.DMA((S // TQ,)),
            pltpu.SemaphoreType.DMA((S // TQ + 1,)),
            pltpu.SemaphoreType.DMA((8,)),
        ],
        compiler_params=pltpu.CompilerParams(vmem_limit_bytes=100 * 2**20),
    )(x, A_wqkv, A_wo, B_w1, B_b1, B_w2, B_b2)
    return out.reshape(B, S, D)
```
